```python
import jax
import jax.numpy as jnp

def _softmax(x, axis=-1):
    return jax.nn.softmax(x, axis=axis)
def _gelu(x):
    return jax.nn.gelu(x, approximate=True)
def _silu(x):
    return jax.nn.silu(x)
def _sigmoid(x):
    return jax.nn.sigmoid(x)
def _layernorm(x, axis=-1, eps=1e-5):
    m = jnp.mean(x, axis=axis, keepdims=True)
    v = jnp.var(x, axis=axis, keepdims=True)
    return (x - m) / jnp.sqrt(v + eps)
def _scatter_add(tgt, idx, src, axis=0):
    return tgt.at[idx].add(src)
def _segment_sum(src, seg, n):
    return jax.ops.segment_sum(src, seg, n)
class _Rng:
    def __init__(self, key):
        self._k = key
    def _next(self):
        self._k, sub = jax.random.split(self._k)
        return sub
    def normal(self, shape):
        return jax.random.normal(self._next(), shape, dtype=jnp.bfloat16)
    def randint(self, lo, hi, shape):
        return jax.random.randint(self._next(), shape, lo, hi, dtype=jnp.int32)
    def uniform(self, shape, lo=0.0, hi=1.0):
        return jax.random.uniform(self._next(), shape, jnp.bfloat16, lo, hi)
    def permutation(self, n):
        return jax.random.permutation(self._next(), n)


kernel_name = 'gated_mix__sliding_block_cached__dense_activation_gelu__decode'

def setup_inputs():
    _rng = _Rng(jax.random.key(int.from_bytes(__import__("os").urandom(4), "little")))
    _w = (lambda a: (lambda t: t.astype(jnp.bfloat16) if jnp.issubdtype(t.dtype, jnp.floating) else t)(jnp.asarray(a)))
    def _A_setup():
        B, Sq, D = 1, 1, 640
        Hq, Hkv, Sk, Dh = 32, 32, 32768, 192
        assert Hq % Hkv == 0, (Hq, Hkv)
        return {
            "x": _w((lambda *s: _rng.normal(s) * 0.05)(B, Sq, D)),
            "k_cache": _w((lambda *s: _rng.normal(s) * 0.05)(B, Hkv, Sk, Dh)),
            "v_cache": _w((lambda *s: _rng.normal(s) * 0.05)(B, Hkv, Sk, Dh)),
            "wq": _w((lambda *s: _rng.normal(s) * 0.05)(D, Hq * Dh) * (D ** -0.5)),
            "wo": _w((lambda *s: _rng.normal(s) * 0.05)(Hq * Dh, D) * ((Hq * Dh) ** -0.5)),
        }
    _A_in = _A_setup()

    def _B_setup():
        B, S, D, F = 1, 1, 640, 1536
        return {
            "x": _w((lambda *s: _rng.normal(s) * 0.05)(B, S, D)),
            "w1": _w((lambda *s: _rng.normal(s) * 0.05)(D, F) * (D ** -0.5)),
            "b1": _w((lambda *s: _rng.normal(s) * 0.05)(F) * 0.01),
            "w2": _w((lambda *s: _rng.normal(s) * 0.05)(F, D) * (F ** -0.5)),
            "b2": _w((lambda *s: _rng.normal(s) * 0.05)(D) * 0.01),
        }
    _B_in = _B_setup()

    return {
        "A_x": _A_in["x"],
        "A_k_cache": _A_in["k_cache"],
        "A_v_cache": _A_in["v_cache"],
        "A_wq": _A_in["wq"],
        "A_wo": _A_in["wo"],
        "B_x": _B_in["x"],
        "B_w1": _B_in["w1"],
        "B_b1": _B_in["b1"],
        "B_w2": _B_in["w2"],
        "B_b2": _B_in["b2"],
        "gate_w": _w((lambda *s: _rng.normal(s) * 0.05)(640)),
    }

def reference(A_x, A_k_cache, A_v_cache, A_wq, A_wo, B_x, B_w1, B_b1, B_w2, B_b2, gate_w):
    def _A_ref(x, k_cache, v_cache, wq, wo):
        B, Sq, D = x.shape
        Hq, Dh = 32, 192
        Hkv, Sk = k_cache.shape[1], k_cache.shape[2]
        W = min(4096, max(256, Sk // 4))
        rep = Hq // Hkv
        q = (lambda x, *d: x.transpose(*d))((x @ wq).reshape(B, Sq, Hq, Dh), 0, 2, 1, 3)
        k = jnp.repeat(k_cache[:, :, Sk - W:, :], rep, axis=1)
        v = jnp.repeat(v_cache[:, :, Sk - W:, :], rep, axis=1)
        scores = jnp.einsum("bhqd,bhkd->bhqk", q, k) * (Dh ** -0.5)
        p = _softmax(scores, axis=-1)
        o = jnp.einsum("bhqk,bhkd->bhqd", p, v)
        return (lambda x, *d: x.transpose(*d))(o, 0, 2, 1, 3).reshape(B, Sq, Hq * Dh) @ wo

    def _B_ref(x, w1, b1, w2, b2):
        h = jnp.einsum("bsd,df->bsf", x, w1) + b1
        h = _gelu(h)
        return jnp.einsum("bsf,fd->bsd", h, w2) + b2

    x = A_x
    g = _sigmoid((x * gate_w).sum(-1, keepdims=True))
    a = _A_ref(x, A_k_cache, A_v_cache, A_wq, A_wo)
    b = _B_ref(x, B_w1, B_b1, B_w2, B_b2)
    return g * a + (1 - g) * b
```

```python
import jax
import jax.numpy as jnp
import jax.experimental.pallas as pl
import jax.experimental.pallas.tpu as pltpu


def _gelu_tanh(h):
    return 0.5 * h * (1.0 + jnp.tanh(0.7978845608028654 * (h + 0.044715 * (h * h * h))))


@jax.jit
def pallas_gated_mix__sliding_block_cached__dense_activation_gelu__decode_kernel(
    A_x: jax.Array,
    A_k_cache: jax.Array,
    A_v_cache: jax.Array,
    A_wq: jax.Array,
    A_wo: jax.Array,
    B_x: jax.Array,
    B_w1: jax.Array,
    B_b1: jax.Array,
    B_w2: jax.Array,
    B_b2: jax.Array,
    gate_w: jax.Array,
):
    _, _, D = A_x.shape
    _, H, SK, DH = A_k_cache.shape
    F = B_w1.shape[1]
    W = min(4096, max(256, SK // 4))
    HP = H // 2
    last = SK // W - 1

    def kernel_function(xa_ref, gw_ref, b1_ref, b2_ref, wq_ref, wo_ref, k_ref, v_ref,
                        w1_ref, w2_ref, o_ref, acc_a, acc_b):
        i = pl.program_id(0)

        @pl.when(i == 0)
        def _():
            acc_a[...] = jnp.zeros_like(acc_a)
            xb = jnp.broadcast_to(xa_ref[0], (8, D))
            h = jnp.dot(xb, w1_ref[...], preferred_element_type=jnp.float32)
            h = h + b1_ref[...].astype(jnp.float32).reshape(1, F)
            h = _gelu_tanh(h)
            acc_b[...] = jnp.dot(h.astype(jnp.bfloat16), w2_ref[...],
                                 preferred_element_type=jnp.float32)

        xa = jnp.broadcast_to(xa_ref[0], (8, D))
        q = jnp.dot(xa, wq_ref[...], preferred_element_type=jnp.float32)
        row = jax.lax.broadcasted_iota(jnp.int32, (8, 2 * DH), 0)
        col = jax.lax.broadcasted_iota(jnp.int32, (8, 2 * DH), 1)
        sel = (row % 2) == (col // DH)
        qm = jnp.where(sel, q, 0.0).astype(jnp.bfloat16)
        s = jnp.dot(qm, k_ref[0], preferred_element_type=jnp.float32) * (DH ** -0.5)
        m = jnp.max(s, axis=-1, keepdims=True)
        p = jnp.exp(s - m)
        l = jnp.sum(p, axis=-1, keepdims=True)
        o = jax.lax.dot_general(p.astype(jnp.bfloat16), v_ref[0], (((1,), (1,)), ((), ())),
                                preferred_element_type=jnp.float32)
        o = o / l
        o = jnp.where(jnp.logical_and(sel, row < 2), o, 0.0)
        o = jnp.sum(o, axis=0, keepdims=True)
        o = jnp.broadcast_to(o, (8, 2 * DH)).astype(jnp.bfloat16)
        acc_a[...] += jnp.dot(o, wo_ref[...], preferred_element_type=jnp.float32)

        @pl.when(i == pl.num_programs(0) - 1)
        def _():
            x = xa_ref[0].astype(jnp.float32)
            gw = gw_ref[...].astype(jnp.float32).reshape(1, D)
            g = jax.nn.sigmoid(jnp.sum(x * gw, axis=-1, keepdims=True))
            b = acc_b[0:1, :] + b2_ref[...].astype(jnp.float32).reshape(1, D)
            o_ref[0] = (g * acc_a[0:1, :] + (1.0 - g) * b).astype(o_ref.dtype)

    kt = jnp.swapaxes(A_k_cache, 2, 3).reshape(HP, 2 * DH, SK)
    vt = jnp.swapaxes(A_v_cache, 2, 3).reshape(HP, 2 * DH, SK)

    def full(a):
        return pl.BlockSpec(a.shape, lambda i: (0,) * a.ndim)

    return pl.pallas_call(
        kernel_function,
        grid=(HP,),
        in_specs=[full(A_x), full(gate_w), full(B_b1), full(B_b2),
                  pl.BlockSpec((D, 2 * DH), lambda i: (0, i)),
                  pl.BlockSpec((2 * DH, D), lambda i: (i, 0)),
                  pl.BlockSpec((1, 2 * DH, W), lambda i: (i, 0, last)),
                  pl.BlockSpec((1, 2 * DH, W), lambda i: (i, 0, last)),
                  full(B_w1), full(B_w2)],
        out_specs=pl.BlockSpec((1, 1, D), lambda i: (0, 0, 0)),
        out_shape=jax.ShapeDtypeStruct((1, 1, D), A_x.dtype),
        scratch_shapes=[pltpu.VMEM((8, D), jnp.float32), pltpu.VMEM((8, D), jnp.float32)],
        compiler_params=pltpu.CompilerParams(dimension_semantics=("arbitrary",),
                                             vmem_limit_bytes=64 << 20),
    )(A_x, gate_w, B_b1, B_b2, A_wq, A_wo, kt, vt, B_w1, B_w2)
```

```python
import functools

import jax
import jax.numpy as jnp
import jax.experimental.pallas as pl
import jax.experimental.pallas.tpu as pltpu

LOOKAHEAD = 7
GROUP_COLS = 2048
WO_ROWS = 8


def _gelu_tanh(h):
    return 0.5 * h * (1.0 + jnp.tanh(0.7978845608028654 * (h + 0.044715 * (h * h * h))))


@jax.jit
def pallas_gated_mix__sliding_block_cached__dense_activation_gelu__decode_kernel(
    A_x: jax.Array,
    A_k_cache: jax.Array,
    A_v_cache: jax.Array,
    A_wq: jax.Array,
    A_wo: jax.Array,
    B_x: jax.Array,
    B_w1: jax.Array,
    B_b1: jax.Array,
    B_w2: jax.Array,
    B_b2: jax.Array,
    gate_w: jax.Array,
):
    del B_x
    f32, bf16 = jnp.float32, jnp.bfloat16
    _, _, D = A_x.shape
    _, H, SK, DH = A_k_cache.shape
    F = B_w1.shape[1]
    W = min(4096, max(256, SK // 4))
    R = H * DH
    C0 = SK - W
    HP = H // 2
    PR = 2 * DH
    L, gc, wr = LOOKAHEAD, GROUP_COLS, WO_ROWS
    ncg = W // gc
    nt = PR // 128

    pro = [("wq", cb, rg) for cb in range(R // gc) for rg in range(D // 128)]
    pro += [("w1", 0, rg) for rg in range(D // 128)]
    pro += [("w2", 0, j) for j in range(F // 128)]
    body = [("k", cg, t) for cg in range(ncg) for t in range(nt)]
    body += [("v", cg, t) for cg in range(ncg) for t in range(nt)]
    body += [("wo", 0, t) for t in range(nt)]
    NP, NB = len(pro), len(body)
    assert L < NB

    def kernel_function(x_hbm, gw_hbm, b1_hbm, b2_hbm, wq_hbm, wo_hbm, k_hbm, v_hbm, w1_hbm, w2_hbm,
                        o_ref, x_v, gw_v, b1_v, b2_v, wq_v, w1_v, w2_v, k_v, v_v, wo_v, q_s, acc_s,
                        psem, bsem, ssem):
        small = [pltpu.make_async_copy(x_hbm, x_v, ssem.at[0]),
                 pltpu.make_async_copy(gw_hbm, gw_v, ssem.at[1]),
                 pltpu.make_async_copy(b1_hbm, b1_v, ssem.at[2]),
                 pltpu.make_async_copy(b2_hbm, b2_v, ssem.at[3])]

        def group(kind, a, b, hp, idx):
            if kind == "wq":
                dst, sem = wq_v.at[pl.ds(b * 128, 128), pl.ds(a * gc, gc)], psem.at[idx]
                cs = [(wq_hbm.at[pl.ds(b * 128 + i * 8, 8), pl.ds(a * gc, gc)],
                       wq_v.at[pl.ds(b * 128 + i * 8, 8), pl.ds(a * gc, gc)], i % 2) for i in range(16)]
            elif kind == "w1":
                dst, sem = w1_v.at[pl.ds(b * 128, 128), :], psem.at[idx]
                cs = [(w1_hbm.at[pl.ds(b * 128 + i * 8, 8), :],
                       w1_v.at[pl.ds(b * 128 + i * 8, 8), :], i % 2) for i in range(16)]
            elif kind == "w2":
                dst, sem = w2_v.at[pl.ds(b * 128, 128), :], psem.at[idx]
                cs = [(w2_hbm.at[pl.ds(b * 128 + i * wr, wr), :],
                       w2_v.at[pl.ds(b * 128 + i * wr, wr), :], i % 2) for i in range(128 // wr)]
            elif kind in ("k", "v"):
                src, buf = (k_hbm, k_v) if kind == "k" else (v_hbm, v_v)
                slot = a * nt + b
                dst, sem = buf.at[slot], bsem.at[idx]
                cs = [(src.at[pl.ds(pl.multiple_of(hp * PR + b * 128 + i * 8, 8), 8), pl.ds(C0 + a * gc, gc)],
                       buf.at[slot, pl.ds(i * 8, 8), :], i % 2) for i in range(16)]
            else:
                dst, sem = wo_v.at[b], bsem.at[idx]
                cs = [(wo_hbm.at[pl.ds(pl.multiple_of(hp * PR + b * 128 + i * wr, wr), wr), :],
                       wo_v.at[b, pl.ds(i * wr, wr), :], i % 2) for i in range(128 // wr)]
            return dst, sem, cs

        def start(kind, a, b, hp, idx):
            _, sem, cs = group(kind, a, b, hp, idx)
            for src, dst, prio in cs:
                pltpu.make_async_copy(src, dst, sem).start(priority=prio)

        def wait(kind, a, b, hp, idx):
            dst, sem, _ = group(kind, a, b, hp, idx)
            pltpu.make_async_copy(dst, dst, sem).wait()

        def start_flat(i):
            if i < NP:
                start(*pro[i], 0, i)
            else:
                start(*body[i - NP], 0, i - NP)

        small[0].start()
        for i in range(L):
            start_flat(i)
        for c in small[1:]:
            c.start()
        small[0].wait()
        x8 = jnp.broadcast_to(x_v[0], (8, D))

        row = jax.lax.broadcasted_iota(jnp.int32, (8, 128), 0)
        lane = jax.lax.broadcasted_iota(jnp.int32, (8, 128), 1)

        def head_mask(t):
            return (row & 1) == ((t * 128 + lane) >= DH).astype(jnp.int32)

        qacc = hacc = bacc = None
        for i, (kind, a, b) in enumerate(pro):
            wait(kind, a, b, 0, i)
            start_flat(i + L)
            if kind == "wq":
                t = jnp.dot(x8[:, b * 128:(b + 1) * 128],
                            wq_v[b * 128:(b + 1) * 128, a * gc:(a + 1) * gc], preferred_element_type=f32)
                qacc = t if b == 0 else qacc + t
                if b == D // 128 - 1:
                    for tt in range(gc // 128):
                        tg = a * (gc // 128) + tt
                        q_s[tg] = jnp.where(head_mask(tg % nt), qacc[:, tt * 128:(tt + 1) * 128], 0.0)
            elif kind == "w1":
                t = jnp.dot(x8[:, b * 128:(b + 1) * 128], w1_v[b * 128:(b + 1) * 128, :],
                            preferred_element_type=f32)
                hacc = t if b == 0 else hacc + t
                if b == D // 128 - 1:
                    small[2].wait()
                    hacc = _gelu_tanh(hacc + b1_v[...].astype(f32).reshape(1, F)).astype(bf16)
            else:
                t = jnp.dot(hacc[:, b * 128:(b + 1) * 128], w2_v[b * 128:(b + 1) * 128, :],
                            preferred_element_type=f32)
                bacc = t if b == 0 else bacc + t
        small[3].wait()
        small[1].wait()
        bfin = bacc[0:1, :] + b2_v[...].astype(f32).reshape(1, D)
        g = jax.nn.sigmoid(jnp.sum(x_v[0].astype(f32) * gw_v[...].astype(f32).reshape(1, D),
                                   axis=-1, keepdims=True))
        acc_s[0:1, :] = (1.0 - g) * bfin
        acc_s[1:2, :] = jnp.broadcast_to(g, (1, D))
        acc_s[8:16, :] = jnp.zeros((8, D), f32)

        def pair(hp, carry):
            qm = [q_s[hp * nt + t].astype(bf16) for t in range(nt)]
            s = [None] * ncg
            o = [None] * nt
            p = linv = aacc = None
            for i, (kind, a, b) in enumerate(body):
                wait(kind, a, b, hp, i)
                nx = i + L
                if nx < NB:
                    start(*body[nx], hp, nx)
                else:
                    @pl.when(hp < HP - 1)
                    def _():
                        start(*body[nx - NB], hp + 1, nx - NB)
                if kind == "k":
                    t = jnp.dot(qm[b], k_v[a * nt + b], preferred_element_type=f32)
                    s[a] = t if b == 0 else s[a] + t
                    if a == ncg - 1 and b == nt - 1:
                        sc = [x * (DH ** -0.5) for x in s]
                        m = functools.reduce(jnp.maximum, [jnp.max(x, axis=-1, keepdims=True) for x in sc])
                        e = [jnp.exp(x - m) for x in sc]
                        l = functools.reduce(jnp.add, [jnp.sum(x, axis=-1, keepdims=True) for x in e])
                        linv = 1.0 / l
                        p = [x.astype(bf16) for x in e]
                elif kind == "v":
                    t = jax.lax.dot_general(p[a], v_v[a * nt + b], (((1,), (1,)), ((), ())),
                                            preferred_element_type=f32)
                    o[b] = t if a == 0 else o[b] + t
                else:
                    ob = jnp.where(head_mask(b), o[b] * linv, 0.0).astype(bf16)
                    t = jnp.dot(ob, wo_v[b], preferred_element_type=f32)
                    aacc = t if b == 0 else aacc + t
            acc_s[8:16, :] += aacc
            return carry

        jax.lax.fori_loop(0, HP, pair, None)
        a_fin = acc_s[8:9, :] + acc_s[9:10, :]
        o_ref[0] = (acc_s[1:2, :] * a_fin + acc_s[0:1, :]).astype(o_ref.dtype)

    kt = jnp.swapaxes(A_k_cache, 2, 3).reshape(R, SK)
    vt = jnp.swapaxes(A_v_cache, 2, 3).reshape(R, SK)
    VM = pltpu.VMEM
    return pl.pallas_call(
        kernel_function,
        in_specs=[pl.BlockSpec(memory_space=pl.ANY)] * 10,
        out_specs=pl.BlockSpec(memory_space=pltpu.VMEM),
        out_shape=jax.ShapeDtypeStruct((1, 1, D), A_x.dtype),
        scratch_shapes=[VM((1, 1, D), bf16), VM((D,), bf16), VM((F,), bf16), VM((D,), bf16),
                        VM((D, R), bf16), VM((D, F), bf16), VM((F, D), bf16),
                        VM((nt * ncg, 128, gc), bf16), VM((nt * ncg, 128, gc), bf16),
                        VM((nt, 128, D), bf16),
                        VM((R // 128, 8, 128), f32), VM((16, D), f32),
                        pltpu.SemaphoreType.DMA((NP,)), pltpu.SemaphoreType.DMA((NB,)),
                        pltpu.SemaphoreType.DMA((4,))],
        compiler_params=pltpu.CompilerParams(vmem_limit_bytes=64 << 20, disable_bounds_checks=True),
    )(A_x, gate_w, B_b1, B_b2, A_wq, A_wo, kt, vt, B_w1, B_w2)
```

```python
import jax
import jax.numpy as jnp
import jax.experimental.pallas as pl
import jax.experimental.pallas.tpu as pltpu

LOOKAHEAD = 7
GROUP = 16
GC = 2048
NF = 4
NQ_STRIDE = 4


def _gelu_tanh(h):
    return 0.5 * h * (1.0 + jnp.tanh(0.7978845608028654 * (h + 0.044715 * (h * h * h))))


def _spread(name, n_copies, rows, per_region):
    return [[(name, (b + k) * rows, rows) for k in range(per_region) if b + k < n_copies]
            for b in range(0, n_copies, per_region)]


@jax.jit
def pallas_gated_mix__sliding_block_cached__dense_activation_gelu__decode_kernel(
    A_x: jax.Array,
    A_k_cache: jax.Array,
    A_v_cache: jax.Array,
    A_wq: jax.Array,
    A_wo: jax.Array,
    B_x: jax.Array,
    B_w1: jax.Array,
    B_b1: jax.Array,
    B_w2: jax.Array,
    B_b2: jax.Array,
    gate_w: jax.Array,
):
    del B_x
    f32, bf16 = jnp.float32, jnp.bfloat16
    _, _, D = A_x.shape
    _, H, SK, DH = A_k_cache.shape
    F = B_w1.shape[1]
    W = min(4096, max(256, SK // 4))
    R = H * DH
    C0 = SK - W
    HP = H // 2
    PR = 2 * DH
    NT = PR // 128
    L = LOOKAHEAD
    NCG = W // GC
    F0 = F - NF * 128

    pro = []
    nq = NQ_STRIDE
    for cb in range(R // GC):
        for s in range(nq):
            pro.append([("wq", (s + nq * k) * 8, 8, cb * GC, GC) for k in range(D // 8 // nq)])
    NQ = len(pro)
    regions = (_spread("wo", (R - PR) // 24, 24, 20) + _spread("w1", D // 8, 8, 16)
               + _spread("w2", F0 // 16, 16, 16))
    flat = [reg[j] for j in range(max(map(len, regions))) for reg in regions if j < len(reg)]
    width = dict(wo=D, w1=F, w2=D)
    for g0 in range(0, len(flat), GROUP):
        pro.append([(a, r, n, 0, width[a]) for a, r, n in flat[g0:g0 + GROUP]])
    NP = len(pro)
    body = [("k", cg, t) for cg in range(NCG) for t in range(NT)]
    body += [("v", cg, t) for cg in range(NCG) for t in range(NT)]
    NB = len(body)
    NE = NT + NF
    assert NE <= L < NB and L < NP
    NPS = L + 1

    def kernel_function(x_hbm, gw_hbm, b1_hbm, b2_hbm, wq_hbm, wo_hbm, k_hbm, v_hbm, w1_hbm, w2_hbm,
                        o_ref, x_v, gw_v, b1_v, b2_v, wq_v, w1_v, w2_v, wo_v, k_v, v_v,
                        q_s, s_s, p_s, o_s, acc_s, hs_s, psem, bsem, esem, ssem):
        arrays = dict(wq=(wq_hbm, wq_v), wo=(wo_hbm, wo_v), w1=(w1_hbm, w1_v), w2=(w2_hbm, w2_v))
        small = [pltpu.make_async_copy(x_hbm, x_v, ssem.at[0]),
                 pltpu.make_async_copy(gw_hbm, gw_v, ssem.at[1]),
                 pltpu.make_async_copy(b1_hbm, b1_v, ssem.at[2]),
                 pltpu.make_async_copy(b2_hbm, b2_v, ssem.at[3])]

        def pro_copies(i):
            out = []
            for n, (a, r0, nr, c0, nc) in enumerate(pro[i]):
                src, dst = arrays[a]
                out.append((pltpu.make_async_copy(src.at[pl.ds(r0, nr), pl.ds(c0, nc)],
                                                  dst.at[pl.ds(r0, nr), pl.ds(c0, nc)],
                                                  psem.at[i % NPS]), n % 2))
            return out

        def start_body(hp, i):
            kind, a, b = body[i]
            src, buf = (k_hbm, k_v) if kind == "k" else (v_hbm, v_v)
            for n in range(GROUP):
                r0 = hp * PR + b * 128 + n * 8
                if not isinstance(r0, int):
                    r0 = pl.multiple_of(r0, 8)
                pltpu.make_async_copy(src.at[pl.ds(r0, 8), pl.ds(C0 + a * GC, GC)],
                                      buf.at[a * NT + b, pl.ds(n * 8, 8), :],
                                      bsem.at[i]).start(priority=n % 2)

        def wait_body(i):
            kind, a, b = body[i]
            dst = (k_v if kind == "k" else v_v).at[a * NT + b]
            pltpu.make_async_copy(dst, dst, bsem.at[i]).wait()

        def epi(t):
            if t < NT:
                return wo_hbm, wo_v, R - PR + t * 128, 16
            return w2_hbm, w2_v, F0 + (t - NT) * 128, 8

        def start_epi(t):
            src, dst, r, cr = epi(t)
            for n in range(128 // cr):
                pltpu.make_async_copy(src.at[pl.ds(r + n * cr, cr), :], dst.at[pl.ds(r + n * cr, cr), :],
                                      esem.at[t]).start(priority=n % 2)

        def wait_epi(t):
            _, dst, r, _ = epi(t)
            v = dst.at[pl.ds(r, 128), :]
            pltpu.make_async_copy(v, v, esem.at[t]).wait()

        def start_flat(i):
            if i < NP:
                for c, prio in pro_copies(i):
                    c.start(priority=prio)
            else:
                start_body(0, i - NP)

        for i in range(L):
            start_flat(i)
            if i == 1:
                for c in small:
                    c.start()

        row = jax.lax.broadcasted_iota(jnp.int32, (8, 128), 0)
        lane = jax.lax.broadcasted_iota(jnp.int32, (8, 128), 1)

        def head_mask(t):
            return (row & 1) == ((t * 128 + lane) >= DH).astype(jnp.int32)

        x8 = None
        for i in range(NP):
            for c, _ in pro_copies(i):
                c.wait()
            start_flat(i + L)
            if i == 0:
                for c in small:
                    c.wait()
                x8 = jnp.broadcast_to(x_v[0], (8, D))
                logit = jnp.sum(x_v[0].astype(f32) * gw_v[...].astype(f32).reshape(1, D),
                                axis=-1, keepdims=True)
                acc_s[1:2, :] = jnp.broadcast_to(jax.nn.sigmoid(logit), (1, D))
                acc_s[8:16, :] = jnp.zeros((8, D), f32)
            if i < NQ and i % nq == nq - 1:
                cb = i // nq
                q = jnp.dot(x8, wq_v[:, cb * GC:(cb + 1) * GC], preferred_element_type=f32)
                for tt in range(GC // 128):
                    tg = cb * (GC // 128) + tt
                    q_s[tg] = jnp.where(head_mask(tg % NT), q[:, tt * 128:(tt + 1) * 128], 0.0)
        h = jnp.dot(x8, w1_v[...], preferred_element_type=f32) + b1_v[...].astype(f32).reshape(1, F)
        h = _gelu_tanh(h).astype(bf16)
        acc_s[0:1, :] = (jnp.dot(h[:, :F0], w2_v[0:F0, :], preferred_element_type=f32)[0:1, :]
                         + b2_v[...].astype(f32).reshape(1, D))
        hf = h.astype(f32)
        for j in range(NF):
            hs_s[j] = jnp.broadcast_to(hf[0:1, F0 + j * 128:F0 + (j + 1) * 128], (128, 128)).T
        o_s[0:NT] = jnp.zeros((NT, 8, 128), f32)

        def out_proj(r0):
            acc = None
            for t in range(NT):
                rr = r0 + t * 128
                if not isinstance(rr, int):
                    rr = pl.multiple_of(rr, 128)
                d = jnp.dot(o_s[t].astype(bf16), wo_v[pl.ds(rr, 128), :], preferred_element_type=f32)
                acc = d if acc is None else acc + d
            acc_s[8:16, :] += acc

        def pair(hp, last):
            for i, (kind, a, b) in enumerate(body):
                wait_body(i)
                nx = i + L
                if nx < NB:
                    start_body(hp, nx)
                elif not last:
                    start_body(hp + 1, nx - NB)
                elif nx - NB < NE:
                    start_epi(nx - NB)
                if i == 0:
                    out_proj(max(hp - 1, 0) * PR if isinstance(hp, int) else jnp.maximum(hp - 1, 0) * PR)
                cols = slice(a * GC, (a + 1) * GC)
                if kind == "k":
                    t = jnp.dot(q_s[hp * NT + b].astype(bf16), k_v[a * NT + b], preferred_element_type=f32)
                    if b == 0:
                        s_s[:, cols] = t
                    elif b < NT - 1:
                        s_s[:, cols] += t
                    else:
                        s_s[:, cols] = (s_s[:, cols] + t) * (DH ** -0.5)
                    if a == NCG - 1 and b == NT - 1:
                        s = s_s[...]
                        e = jnp.exp(s - jnp.max(s, axis=-1, keepdims=True))
                        p_s[...] = e.astype(bf16)
                        o_s[NT] = jnp.broadcast_to(1.0 / jnp.sum(e, axis=-1, keepdims=True), (8, 128))
                else:
                    t = jax.lax.dot_general(p_s[:, cols], v_v[a * NT + b], (((1,), (1,)), ((), ())),
                                            preferred_element_type=f32)
                    if a < NCG - 1:
                        o_s[NT + 1 + b] = t if a == 0 else o_s[NT + 1 + b] + t
                    else:
                        o_s[b] = jnp.where(head_mask(b), (o_s[NT + 1 + b] + t) * o_s[NT], 0.0)

        def step(hp, carry):
            pair(hp, False)
            return carry

        jax.lax.fori_loop(0, HP - 1, step, 0)
        pair(HP - 1, True)

        for t in range(NE):
            wait_epi(t)
            if t < NT:
                r = R - PR + t * 128
                acc_s[8:16, :] += jnp.dot(o_s[t].astype(bf16), wo_v[r:r + 128, :],
                                          preferred_element_type=f32)
            else:
                j = t - NT
                parts = []
                for c in range(D // 128):
                    w = w2_v[F0 + j * 128:F0 + (j + 1) * 128, c * 128:(c + 1) * 128].astype(f32)
                    parts.append((w * hs_s[j]).reshape(16, 8, 128).sum(axis=0))
                pv = jnp.concatenate(parts, axis=1)
                if j == 0:
                    acc_s[16:24, :] = pv
                else:
                    acc_s[16:24, :] += pv
        g = acc_s[1:2, :]
        a_out = acc_s[8:9, :] + acc_s[9:10, :]
        b_out = acc_s[0:1, :] + jnp.sum(acc_s[16:24, :], axis=0, keepdims=True)
        o_ref[0] = (g * a_out + (1.0 - g) * b_out).astype(o_ref.dtype)

    kt = jnp.swapaxes(A_k_cache, 2, 3).reshape(R, SK)
    vt = jnp.swapaxes(A_v_cache, 2, 3).reshape(R, SK)
    VM = pltpu.VMEM
    return pl.pallas_call(
        kernel_function,
        in_specs=[pl.BlockSpec(memory_space=pl.ANY)] * 10,
        out_specs=pl.BlockSpec(memory_space=pltpu.VMEM),
        out_shape=jax.ShapeDtypeStruct((1, 1, D), A_x.dtype),
        scratch_shapes=[VM((1, 1, D), bf16), VM((D,), bf16), VM((F,), bf16), VM((D,), bf16),
                        VM((D, R), bf16), VM((D, F), bf16), VM((F, D), bf16), VM((R, D), bf16),
                        VM((NT * NCG, 128, GC), bf16), VM((NT * NCG, 128, GC), bf16),
                        VM((R // 128, 8, 128), f32), VM((8, W), f32), VM((8, W), bf16),
                        VM((2 * NT + 1, 8, 128), f32), VM((24, D), f32), VM((NF, 128, 128), f32),
                        pltpu.SemaphoreType.DMA((NPS,)), pltpu.SemaphoreType.DMA((NB,)),
                        pltpu.SemaphoreType.DMA((NE,)), pltpu.SemaphoreType.DMA((4,))],
        compiler_params=pltpu.CompilerParams(vmem_limit_bytes=64 << 20, disable_semaphore_checks=True),
    )(A_x, gate_w, B_b1, B_b2, A_wq, A_wo, kt, vt, B_w1, B_w2)
```

```python
import jax
import jax.numpy as jnp
import jax.experimental.pallas as pl
import jax.experimental.pallas.tpu as pltpu

LOOKAHEAD = 7
GROUP = 16
GC = 2048
NF = 4
NQ_STRIDE = 4


def _gelu_tanh(h):
    return 0.5 * h * (1.0 + jnp.tanh(0.7978845608028654 * (h + 0.044715 * (h * h * h))))


def _spread(name, n_copies, rows, per_region):
    return [[(name, (b + k) * rows, rows) for k in range(per_region) if b + k < n_copies]
            for b in range(0, n_copies, per_region)]


@jax.jit
def pallas_gated_mix__sliding_block_cached__dense_activation_gelu__decode_kernel(
    A_x: jax.Array,
    A_k_cache: jax.Array,
    A_v_cache: jax.Array,
    A_wq: jax.Array,
    A_wo: jax.Array,
    B_x: jax.Array,
    B_w1: jax.Array,
    B_b1: jax.Array,
    B_w2: jax.Array,
    B_b2: jax.Array,
    gate_w: jax.Array,
):
    del B_x
    f32, bf16 = jnp.float32, jnp.bfloat16
    _, _, D = A_x.shape
    _, H, SK, DH = A_k_cache.shape
    F = B_w1.shape[1]
    W = min(4096, max(256, SK // 4))
    R = H * DH
    C0 = SK - W
    HP = H // 2
    PR = 2 * DH
    NT = PR // 128
    L = LOOKAHEAD
    NCG = W // GC
    F0 = F - NF * 128

    pro = []
    nq = NQ_STRIDE
    for cb in range(R // GC):
        for s in range(nq):
            pro.append([("wq", (s + nq * k) * 8, 8, cb * GC, GC) for k in range(D // 8 // nq)])
    NQ = len(pro)
    regions = (_spread("wo", (R - PR) // 24, 24, 20) + _spread("w1", D // 8, 8, 16)
               + _spread("w2", F0 // 16, 16, 16))
    flat = [reg[j] for j in range(max(map(len, regions))) for reg in regions if j < len(reg)]
    width = dict(wo=D, w1=F, w2=D)
    for g0 in range(0, len(flat), GROUP):
        pro.append([(a, r, n, 0, width[a]) for a, r, n in flat[g0:g0 + GROUP]])
    NP = len(pro)
    body = [("k", cg, t) for cg in range(NCG) for t in range(NT)]
    body += [("v", cg, t) for cg in range(NCG) for t in range(NT)]
    NB = len(body)
    NE = NT + NF
    assert NE <= L and L + 1 < NB and L < NP

    def kernel_function(x_hbm, gw_hbm, b1_hbm, b2_hbm, wq_hbm, wo_hbm, k_hbm, v_hbm, w1_hbm, w2_hbm,
                        o_ref, x_v, gw_v, b1_v, b2_v, wq_v, w1_v, w2_v, wo_v, k_v, v_v,
                        q_s, s_s, p_s, o_s, acc_s, hs_s, sems):
        arrays = dict(wq=(wq_hbm, wq_v), wo=(wo_hbm, wo_v), w1=(w1_hbm, w1_v), w2=(w2_hbm, w2_v))
        small = [pltpu.make_async_copy(src, dst, sems.at[NB - 1])
                 for src, dst in ((x_hbm, x_v), (gw_hbm, gw_v), (b1_hbm, b1_v), (b2_hbm, b2_v))]

        def pro_copies(i):
            out = []
            for n, (a, r0, nr, c0, nc) in enumerate(pro[i]):
                src, dst = arrays[a]
                out.append((pltpu.make_async_copy(src.at[pl.ds(r0, nr), pl.ds(c0, nc)],
                                                  dst.at[pl.ds(r0, nr), pl.ds(c0, nc)],
                                                  sems.at[i % NB]), n % 2))
            return out

        def start_body(hp, i):
            kind, a, b = body[i]
            src, buf = (k_hbm, k_v) if kind == "k" else (v_hbm, v_v)
            for n in range(GROUP):
                r0 = hp * PR + b * 128 + n * 8
                if not isinstance(r0, int):
                    r0 = pl.multiple_of(r0, 8)
                pltpu.make_async_copy(src.at[pl.ds(r0, 8), pl.ds(C0 + a * GC, GC)],
                                      buf.at[a * NT + b, pl.ds(n * 8, 8), :],
                                      sems.at[(NP + i) % NB]).start(priority=n % 2)

        def wait_body(i):
            kind, a, b = body[i]
            dst = (k_v if kind == "k" else v_v).at[a * NT + b]
            pltpu.make_async_copy(dst, dst, sems.at[(NP + i) % NB]).wait()

        def epi(t):
            if t < NT:
                return wo_hbm, wo_v, R - PR + t * 128, 16
            return w2_hbm, w2_v, F0 + (t - NT) * 128, 8

        def start_epi(t):
            src, dst, r, cr = epi(t)
            for n in range(128 // cr):
                pltpu.make_async_copy(src.at[pl.ds(r + n * cr, cr), :], dst.at[pl.ds(r + n * cr, cr), :],
                                      sems.at[(NP + t) % NB]).start(priority=n % 2)

        def wait_epi(t):
            _, dst, r, _ = epi(t)
            v = dst.at[pl.ds(r, 128), :]
            pltpu.make_async_copy(v, v, sems.at[(NP + t) % NB]).wait()

        def start_flat(i):
            if i < NP:
                for c, prio in pro_copies(i):
                    c.start(priority=prio)
            else:
                start_body(0, i - NP)

        for i in range(L):
            start_flat(i)
            if i == 1:
                for c in small:
                    c.start()

        row = jax.lax.broadcasted_iota(jnp.int32, (8, 128), 0)
        lane = jax.lax.broadcasted_iota(jnp.int32, (8, 128), 1)

        def head_mask(t):
            return (row & 1) == ((t * 128 + lane) >= DH).astype(jnp.int32)

        x8 = None
        for i in range(NP):
            for c, _ in pro_copies(i):
                c.wait()
            start_flat(i + L)
            if i == 0:
                for c in small:
                    c.wait()
                x8 = jnp.broadcast_to(x_v[0], (8, D))
                logit = jnp.sum(x_v[0].astype(f32) * gw_v[...].astype(f32).reshape(1, D),
                                axis=-1, keepdims=True)
                acc_s[1:2, :] = jnp.broadcast_to(jax.nn.sigmoid(logit), (1, D))
                acc_s[8:16, :] = jnp.zeros((8, D), f32)
            if i < NQ and i % nq == nq - 1:
                cb = i // nq
                q = jnp.dot(x8, wq_v[:, cb * GC:(cb + 1) * GC], preferred_element_type=f32)
                for tt in range(GC // 128):
                    tg = cb * (GC // 128) + tt
                    q_s[tg] = jnp.where(head_mask(tg % NT), q[:, tt * 128:(tt + 1) * 128], 0.0)
        h = jnp.dot(x8, w1_v[...], preferred_element_type=f32) + b1_v[...].astype(f32).reshape(1, F)
        h = _gelu_tanh(h).astype(bf16)
        acc_s[0:1, :] = (jnp.dot(h[:, :F0], w2_v[0:F0, :], preferred_element_type=f32)[0:1, :]
                         + b2_v[...].astype(f32).reshape(1, D))
        hf = h.astype(f32)
        for j in range(NF):
            hs_s[j] = jnp.broadcast_to(hf[0:1, F0 + j * 128:F0 + (j + 1) * 128], (128, 128)).T
        o_s[0:NT] = jnp.zeros((NT, 8, 128), f32)

        def out_proj(r0):
            acc = None
            for t in range(NT):
                rr = r0 + t * 128
                if not isinstance(rr, int):
                    rr = pl.multiple_of(rr, 128)
                d = jnp.dot(o_s[t].astype(bf16), wo_v[pl.ds(rr, 128), :], preferred_element_type=f32)
                acc = d if acc is None else acc + d
            acc_s[8:16, :] += acc

        def pair(hp, last):
            for i, (kind, a, b) in enumerate(body):
                wait_body(i)
                nx = i + L
                if nx < NB:
                    start_body(hp, nx)
                elif not last:
                    start_body(hp + 1, nx - NB)
                elif nx - NB < NE:
                    start_epi(nx - NB)
                if i == 0:
                    out_proj(max(hp - 1, 0) * PR if isinstance(hp, int) else jnp.maximum(hp - 1, 0) * PR)
                cols = slice(a * GC, (a + 1) * GC)
                if kind == "k":
                    t = jnp.dot(q_s[hp * NT + b].astype(bf16), k_v[a * NT + b], preferred_element_type=f32)
                    if b == 0:
                        s_s[:, cols] = t
                    elif b < NT - 1:
                        s_s[:, cols] += t
                    else:
                        s_s[:, cols] = (s_s[:, cols] + t) * (DH ** -0.5)
                    if a == NCG - 1 and b == NT - 1:
                        s = s_s[...]
                        e = jnp.exp(s - jnp.max(s, axis=-1, keepdims=True))
                        p_s[...] = e.astype(bf16)
                        o_s[NT] = jnp.broadcast_to(1.0 / jnp.sum(e, axis=-1, keepdims=True), (8, 128))
                else:
                    t = jax.lax.dot_general(p_s[:, cols], v_v[a * NT + b], (((1,), (1,)), ((), ())),
                                            preferred_element_type=f32)
                    if a < NCG - 1:
                        o_s[NT + 1 + b] = t if a == 0 else o_s[NT + 1 + b] + t
                    else:
                        o_s[b] = jnp.where(head_mask(b), (o_s[NT + 1 + b] + t) * o_s[NT], 0.0)

        def step(hp, carry):
            pair(hp, False)
            return carry

        jax.lax.fori_loop(0, HP - 1, step, 0)
        pair(HP - 1, True)

        for t in range(NE):
            wait_epi(t)
            if t < NT:
                r = R - PR + t * 128
                acc_s[8:16, :] += jnp.dot(o_s[t].astype(bf16), wo_v[r:r + 128, :],
                                          preferred_element_type=f32)
            else:
                j = t - NT
                parts = []
                for c in range(D // 128):
                    w = w2_v[F0 + j * 128:F0 + (j + 1) * 128, c * 128:(c + 1) * 128].astype(f32)
                    parts.append((w * hs_s[j]).reshape(16, 8, 128).sum(axis=0))
                pv = jnp.concatenate(parts, axis=1)
                if j == 0:
                    acc_s[16:24, :] = pv
                else:
                    acc_s[16:24, :] += pv
        g = acc_s[1:2, :]
        a_out = acc_s[8:9, :] + acc_s[9:10, :]
        b_out = acc_s[0:1, :] + jnp.sum(acc_s[16:24, :], axis=0, keepdims=True)
        o_ref[0] = (g * a_out + (1.0 - g) * b_out).astype(o_ref.dtype)

    kt = jnp.swapaxes(A_k_cache, 2, 3).reshape(R, SK)
    vt = jnp.swapaxes(A_v_cache, 2, 3).reshape(R, SK)
    VM = pltpu.VMEM
    return pl.pallas_call(
        kernel_function,
        in_specs=[pl.BlockSpec(memory_space=pl.ANY)] * 10,
        out_specs=pl.BlockSpec(memory_space=pltpu.VMEM),
        out_shape=jax.ShapeDtypeStruct((1, 1, D), A_x.dtype),
        scratch_shapes=[VM((1, 1, D), bf16), VM((D,), bf16), VM((F,), bf16), VM((D,), bf16),
                        VM((D, R), bf16), VM((D, F), bf16), VM((F, D), bf16), VM((R, D), bf16),
                        VM((NT * NCG, 128, GC), bf16), VM((NT * NCG, 128, GC), bf16),
                        VM((R // 128, 8, 128), f32), VM((8, W), f32), VM((8, W), bf16),
                        VM((2 * NT + 1, 8, 128), f32), VM((24, D), f32), VM((NF, 128, 128), f32),
                        pltpu.SemaphoreType.DMA((NB,))],
        compiler_params=pltpu.CompilerParams(vmem_limit_bytes=64 << 20),
    )(A_x, gate_w, B_b1, B_b2, A_wq, A_wo, kt, vt, B_w1, B_w2)
```
